```python
import os as _os
_os.environ.setdefault("JAX_PLATFORMS", "cpu")
import jax
import jax.numpy as jnp

def _softmax(x, axis=-1):
    return jax.nn.softmax(x, axis=axis)
def _gelu(x):
    return jax.nn.gelu(x, approximate=True)
def _silu(x):
    return jax.nn.silu(x)
def _sigmoid(x):
    return jax.nn.sigmoid(x)
def _layernorm(x, axis=-1, eps=1e-5):
    m = jnp.mean(x, axis=axis, keepdims=True)
    v = jnp.var(x, axis=axis, keepdims=True)
    return (x - m) / jnp.sqrt(v + eps)
def _scatter_add(tgt, idx, src, axis=0):
    return tgt.at[idx].add(src)
def _segment_sum(src, seg, n):
    return jax.ops.segment_sum(src, seg, n)
class _Rng:
    def __init__(self, key):
        self._k = key
    def _next(self):
        self._k, sub = jax.random.split(self._k)
        return sub
    def normal(self, shape):
        return jax.random.normal(self._next(), shape, dtype=jnp.bfloat16)
    def randint(self, lo, hi, shape):
        return jax.random.randint(self._next(), shape, lo, hi, dtype=jnp.int32)
    def uniform(self, shape, lo=0.0, hi=1.0):
        return jax.random.uniform(self._next(), shape, jnp.bfloat16, lo, hi)
    def permutation(self, n):
        return jax.random.permutation(self._next(), n)


kernel_name = 'interleave_layers__spectral_gfnet__linear_attn_block__prompt'

def setup_inputs():
    _rng = _Rng(jax.random.key(int.from_bytes(__import__("os").urandom(4), "little")))
    _w = (lambda a: (lambda t: t.astype(jnp.bfloat16) if jnp.issubdtype(t.dtype, jnp.floating) else t)(jnp.asarray(a)))
    def _A_setup():
        B, S, D = 1, 2048, 640
        Df = D // 2 + 1
        return {
            "x": _w((lambda *s: _rng.normal(s) * 0.05)(B, S, D)),
            "w_r": _w((lambda *s: _rng.normal(s) * 0.4)(S, Df) * 0.02),
            "w_i": _w((lambda *s: _rng.normal(s) * 0.4)(S, Df) * 0.02),
        }
    _A_in = _A_setup()

    def _B_setup():
        B, S, D = 1, 2048, 640
        return {
            "x": _w((lambda *s: _rng.normal(s) * 0.05)(B, S, D)),
            "wqkv": _w((lambda *s: _rng.normal(s) * 0.05)(D, 3 * D)),
            "wo": _w((lambda *s: _rng.normal(s) * 0.05)(D, D)),
        }
    _B_in = _B_setup()

    return {
        "A_x": _A_in["x"],
        "A_w_r": _A_in["w_r"],
        "A_w_i": _A_in["w_i"],
        "B_x": _B_in["x"],
        "B_wqkv": _B_in["wqkv"],
        "B_wo": _B_in["wo"],
    }

def reference(A_x, A_w_r, A_w_i, B_x, B_wqkv, B_wo):
    def _A_ref(x, w_r, w_i):
        B, S, D = x.shape
        X = (lambda x, axes=(-2,-1): jnp.fft.rfft2(x.astype(jnp.float32), axes=axes))(x, axes=(-2, -1))
        W = w_r + 1j * w_i
        X = X * W
        y = (lambda x, s, axes=(-2,-1): jnp.fft.irfft2(x, s=s, axes=axes).astype(jnp.bfloat16))(X, (S, D), axes=(-2, -1))
        return y

    def _B_ref(x, wqkv, wo):
        B, S, D = x.shape
        H = 32; Dh = D // H
        qkv = (lambda x, *d: x.transpose(*d))((x @ wqkv).reshape(B, S, 3, H, Dh), 2, 0, 3, 1, 4)
        q, k, v = qkv[0], qkv[1], qkv[2]
        phi = lambda t: jnp.where(t > 0, t + 1, jnp.exp(t)) + 1e-6
        pq, pk = phi(q), phi(k)
        kv = jnp.einsum("bhsd,bhse->bhde", pk, v)
        z = jnp.einsum("bhsd->bhd", pk)
        num = jnp.einsum("bhqd,bhde->bhqe", pq, kv)
        den = jnp.einsum("bhqd,bhd->bhq", pq, z)[..., None] + 1e-6
        o = num / den
        return (lambda x, *d: x.transpose(*d))(o, 0, 2, 1, 3).reshape(B, S, D) @ wo

    x = A_x
    x = x + _A_ref(_layernorm(x, axis=-1), A_w_r, A_w_i)
    x = x + _B_ref(_layernorm(x, axis=-1), B_wqkv, B_wo)
    x = x + _A_ref(_layernorm(x, axis=-1), A_w_r, A_w_i)
    x = x + _B_ref(_layernorm(x, axis=-1), B_wqkv, B_wo)
    return x
```

```python
import math

import jax
import jax.numpy as jnp
import numpy as np
from jax import lax
import jax.experimental.pallas as pl
import jax.experimental.pallas.tpu as pltpu

S, D, H = 2048, 640, 32
DH = D // H
DF = D // 2 + 1
R1, R2 = 32, 64
NT = D // 128
NS = R2 // 8
SLAB = R1 * 8
NG = 4
T = S // NG
LN_ROWS = 128
NFWD = 9
TILES = (1, 2, 3, 4, 0)
PACE = 1
LAG = 3
NCLS = R1 // 2
BF, F32, U32 = jnp.bfloat16, jnp.float32, jnp.uint32
RESIDUES = ((0, 5), (6, 4), (1, 9), (2, 8), (7, 3))


def _add(a, b):
    if a[0] == b[0]:
        return (a[0], a[1] + b[1])
    return (1, a[1] - b[1]) if a[0] > 0 else (1, b[1] - a[1])


def _neg(a):
    return (-a[0], a[1])


def _sub(a, b):
    return _add(a, _neg(b))


def _mul(a, c):
    return (a[0] if c > 0 else -a[0], a[1] * abs(c))


def _rot(re, im, k, n):
    c, s = math.cos(2 * math.pi * k / n), math.sin(2 * math.pi * k / n)
    if 8 * abs(k) == n:
        if k > 0:
            return _mul(_sub(re, im), c), _mul(_add(re, im), c)
        return _mul(_add(re, im), c), _mul(_sub(im, re), c)
    return _sub(_mul(re, c), _mul(im, s)), _add(_mul(re, s), _mul(im, c))


def _rfft(x, seen):
    n = len(x)
    if n == 2:
        return [(_add(x[0], x[1]), None), (_sub(x[0], x[1]), None)]
    e, o = _rfft(x[0::2], seen), _rfft(x[1::2], seen)
    out = [None] * (n // 2 + 1)
    out[0] = (_add(e[0][0], o[0][0]), None)
    out[n // 2] = (_sub(e[0][0], o[0][0]), None)
    out[n // 4] = (e[n // 4][0], _neg(o[n // 4][0]))
    for k in range(1, n // 4):
        tr, ti = _rot(o[k][0], o[k][1], -k, n)
        out[k] = (_add(e[k][0], tr), _add(e[k][1], ti))
        out[n // 2 - k] = (_sub(e[k][0], tr), _sub(ti, e[k][1]))
    if n < R1:
        seen += [v[0][1] for v in out[:n // 4]]
    return out


def _rfft_t(z):
    n = 2 * (len(z) - 1)
    if n == 2:
        return [_add(z[0][0], z[1][0]), _sub(z[0][0], z[1][0])]
    e, o = [None] * (n // 4 + 1), [None] * (n // 4 + 1)
    e[0] = (_add(z[0][0], z[n // 2][0]), None)
    o[0] = (_sub(z[0][0], z[n // 2][0]), None)
    e[n // 4] = (z[n // 4][0], None)
    o[n // 4] = (_neg(z[n // 4][1]), None)
    for k in range(1, n // 4):
        a, b = z[k], z[n // 2 - k]
        e[k] = (_add(a[0], b[0]), _sub(a[1], b[1]))
        o[k] = _rot(_sub(a[0], b[0]), _add(a[1], b[1]), k, n)
    x = [None] * n
    x[0::2], x[1::2] = _rfft_t(e), _rfft_t(o)
    return x


def _tok_signed(x, seen):
    z = _rfft([(1, v) for v in x], seen)
    return [z[0][0], z[NCLS][0]] + [v for c in range(1, NCLS) for v in z[c]]


def _tok_fwd(x, seen):
    return [v for _, v in _tok_signed(x, seen)]


def _tok_inv(v):
    v = [(sign, a) for (sign, _), a in zip(_tok_signed([0.0] * R1, []), v)]
    z = [(v[0], None)] + [(v[2 * c], v[2 * c + 1]) for c in range(1, NCLS)] + [(v[1], None)]
    return [a if sign > 0 else -a for sign, a in _rfft_t(z)]


_C5 = math.sqrt(5.0) / 4
_S5 = math.sin(4 * math.pi / 5) / math.sin(2 * math.pi / 5)


def _swap_halves(a, b, lo, where, roll):
    r = roll(where(lo, b, a))
    return where(lo, a, r), where(lo, r, b)


def _radix5(x):
    a1, b1, a2, b2 = x[1] + x[4], x[1] - x[4], x[2] + x[3], x[2] - x[3]
    t = a1 + a2
    m1, m2 = x[0] - 0.25 * t, _C5 * (a1 - a2)
    return x[0] + t, m1 + m2, b1 + _S5 * b2, m1 - m2, _S5 * b1 - b2


def _feat_fwd(x, lo, where, roll):
    y0, r1, i1, r2, i2 = _radix5([where(lo, x[b], x[(b + 2) % 5]) for b in range(5)])
    p1, q1 = _swap_halves(r1, i1, lo, where, roll)
    p2, q2 = _swap_halves(r2, i2, lo, where, roll)
    return [y0, p1 + q1, p1 - q1, p2 + q2, p2 - q2]


def _feat_fwd_halves(x):
    a = _radix5(x[0::2])
    b = _radix5([x[(2 * n + 5) % 10] for n in range(5)])
    out = [a[0], b[0]]
    for n in (1, 3):
        out += [a[n] + b[n], a[n + 1] + b[n + 1], a[n] - b[n], a[n + 1] - b[n + 1]]
    return out


def _feat_inv(y, lo, where, roll):
    r1, i1 = _swap_halves(y[1] + y[2], y[1] - y[2], lo, where, roll)
    r2, i2 = _swap_halves(y[3] + y[4], y[3] - y[4], lo, where, roll)
    m1, m2 = r1 + r2, _C5 * (r1 - r2)
    t = y[0] - 0.25 * m1
    a1, a2 = t + m2, t - m2
    b1, b2 = i1 + _S5 * i2, _S5 * i1 - i2
    x = [y[0] + m1, a1 + b1, a2 + b2, a2 - b2, a1 - b1]
    return [where(lo, x[b], x[(b + 3) % 5]) for b in range(5)]


def _pack_rows(a):
    u = np.asarray(a, np.float32).astype(BF).view(np.uint16).astype(np.uint32)
    return u[..., 0::2, :] | (u[..., 1::2, :] << 16)


def _make_constants():
    lo = np.arange(128) < 64
    roll = lambda a: np.roll(a, 64, axis=1)
    eye = [np.eye(D)[:, 128 * j:128 * (j + 1)] for j in range(NT)]
    bf = np.concatenate(_feat_fwd(eye, lo, np.where, roll), axis=1)
    bi = np.concatenate(_feat_inv(eye, lo, np.where, roll), axis=1)
    cols = []
    for ra, rb in RESIDUES:
        kd = np.stack([ra + 10 * np.arange(32), rb + 10 * np.arange(32)], 1).ravel()
        ang = 2 * np.pi * np.outer(np.arange(D), kd) / D
        re, im = np.cos(ang), -np.sin(ang)
        if ra == 0:
            re[:, 0] = math.sqrt(0.5)
            im[:, 0] = math.sqrt(0.5) * np.cos(np.pi * np.arange(D))
        cols += [re, im]
    fd = np.concatenate(cols, axis=1) * math.sqrt(2.0 / D)
    tf = np.linalg.solve(bf, fd)
    ti = fd.T @ np.linalg.inv(bi)
    blk = lambda m: [m[128 * j:128 * (j + 1), 128 * j:128 * (j + 1)] for j in range(NT)]
    f5 = [fd[:, 0:128]] + [np.concatenate([fd[:, 128 * j + h:][:, :64], fd[:, 128 * j + h + 128:][:, :64]], 1)
                           for j in (1, 3) for h in (0, 64)]
    t5 = np.linalg.solve(np.concatenate(_radix5(eye), axis=1), np.concatenate(f5, axis=1))
    t5 = [t5[:128, :128]] + [t5[128 * (j + a):128 * (j + a + 1), 128 * (j + b):128 * (j + b + 1)]
                             for j in (1, 3) for b in (0, 1) for a in (0, 1)]
    dmat = np.stack(t5 + blk(ti))

    cf = np.linalg.inv(np.stack(_tok_fwd(list(np.eye(R1)), [])))
    s = np.arange(R2)[None, :] + R2 * np.arange(R1)[:, None]
    sf = []
    for c in range(NCLS):
        m = np.arange(R2)
        ks = R1 * m + (c if c else np.where(m < R2 // 2, 0, NCLS))
        ang = 2 * np.pi * ks[:, None, None] * s[None] / S
        f = np.concatenate([np.cos(ang), -np.sin(ang)])
        if c == 0:
            f[R2] = np.cos(np.pi * s)
        sf.append(np.einsum("kab,ar->krb", f, cf[:, 2 * c:2 * c + 2]).reshape(128, 128))
    smat = np.stack(sf)
    return tuple(_pack_rows(a) for a in (smat, dmat))


_SMAT, _DMAT = _make_constants()


def _dot(a, b):
    return jnp.dot(a, b, preferred_element_type=F32)


def _dot_nt(a, b):
    return lax.dot_general(a, b, (((1,), (1,)), ((), ())), preferred_element_type=F32)


def _tile(j):
    return slice(128 * j, 128 * (j + 1))


def _roll64(a):
    return pltpu.roll(a, 64, 1)


def _lanes(rows):
    return lax.broadcasted_iota(jnp.int32, (rows, 128), 1)


def _rows(rows):
    return lax.broadcasted_iota(jnp.int32, (rows, 128), 0)


def _phi(t):
    return jnp.where(t > 0, t + 1.0, jnp.exp(t)) + 1e-6


def _layernorm_scale(x):
    sq = [v * v for v in x]
    ac = jnp.where(_lanes(x[0].shape[0]) != 0, sq[0], 0.0)
    var = jnp.sum(sum(sq[1:], ac), axis=1, keepdims=True) * (1.0 / D)
    return jnp.broadcast_to(lax.rsqrt(var + 1e-5), x[0].shape)


def _regroup(f):
    lo = _lanes(f[0].shape[0]) < 64
    return [f[0], *_swap_halves(f[1], f[2], lo, jnp.where, _roll64),
            *_swap_halves(f[3], f[4], lo, jnp.where, _roll64)]


def _get(ref, *idx, rows=None):
    r = () if rows is None else (pl.ds(rows[0] // 2, rows[1] // 2),)
    return pltpu.bitcast(ref[(*idx, *r)], BF)


def _put(ref, j, v, start=0):
    ref[j, pl.ds(start // 2, v.shape[0] // 2), :] = pltpu.bitcast(v.astype(BF), U32)


def _cat(ref, rows=None):
    return jnp.concatenate([_get(ref, j, rows=rows) for j in range(NT)], axis=1)


def _ds(start, size, align=None):
    if isinstance(start, int):
        return pl.ds(start, size)
    return pl.ds(pl.multiple_of(start, align or size), size)


def _take(gen, n):
    for _ in range(n):
        yield next(gen, None)


def _chain(*gens):
    for gen in gens:
        yield from gen


def _kernel(x_hbm, wr_hbm, wi_hbm, wqkv_hbm, wo_hbm, smat_hbm, dmat_hbm, o_hbm,
            xio, wbuf, wraw, smat, dmat, perm, wpair, coef, coef0,
            xf0, xres, xn, scale, ubuf, vbuf, wqt, wkt, wvf, wof, gacc, rows, mmat, zrow,
            pk, att, wtmp, pq, scale0,
            sem_x, sem_w, sem_o, sem_f):
    def slab_copies(i, which=(0, 1, 2)):
        cols = _ds(i * 256, 256)
        ends = ((x_hbm.at[:, _ds(i * 8, 8), :], xio.at[i]),
                (wr_hbm.at[:, cols], wbuf.at[0, i + 1]), (wi_hbm.at[:, cols], wbuf.at[1, i + 1]))
        return [pltpu.make_async_copy(*ends[n], sem_x.at[n * NS + i]) for n in which]

    parts = [(dmat_hbm.at[pl.ds(0, NFWD)], dmat.at[pl.ds(0, NFWD)]),
             (smat_hbm, smat.at[pl.ds(0, NCLS)]),
             (dmat_hbm.at[pl.ds(NFWD, NT)], dmat.at[pl.ds(NFWD, NT)])]
    parts += [(wqkv_hbm.at[:, pl.ds(i * D + 128 * e, 128)] if i < 3 else
               wo_hbm.at[:, pl.ds(128 * e, 128)], wraw[i].at[e])
              for i in (1, 2, 0, 3) for e in range(NT)]
    w_copy = [pltpu.make_async_copy(src, dst, sem_w.at[i]) for i, (src, dst) in enumerate(parts)]
    parts = [(i, NT - 1, slice(None)) for i in range(NS - 1)]
    parts += [(NS - 1, j, pl.ds(128 * j, 128)) for j in range(NT)]
    o_copy = {(i, j): pltpu.make_async_copy(
        xio.at[i, :, :, cols], o_hbm.at[:, pl.ds(i * 8, 8), cols], sem_o.at[n])
        for n, (i, j, cols) in enumerate(parts)}

    order = {"zero": None, "tokens": [], "pace": None, "results": []}

    def anywhere(ref, sub):
        z = [jnp.clip(order["zero"], 0, n - 1) for n in (*ref.shape[:-2], ref.shape[-2] // sub)]
        return z[:-1], pl.ds(pl.multiple_of(z[-1] * sub, sub), sub)

    def written(ref):
        lead, r = anywhere(ref, 8)
        order["tokens"].append(ref[(*lead, r, slice(0, 128))])
        return order["tokens"][-1]

    def hold(ref, token):
        token = pltpu.bitcast(token, ref.dtype)
        lead, r = anywhere(ref, token.shape[0])
        ref[(ref.shape[0] - 1 - lead[0], *lead[1:], r, slice(0, 128))] = token

    def paced(ref):
        if order["pace"] is not None:
            hold(ref, order["pace"])

    def step_done(src, dst):
        token = written(dst)
        if order["pace"] is None:
            hold(src, token)

    def emit(main, *sides):
        steps = sorted(((i + 0.5) / n, k) for k, (_, n) in enumerate(sides) for i in range(n))
        for i in range(main[1]):
            result = next(main[0], None)
            if result is not None:
                order["results"].append(result)
            result = order["results"][-1 - PACE] if len(order["results"]) > PACE else None
            mine = [k for t, k in steps if int(t * max(main[1] - 1, 1)) == i]
            for n, k in enumerate(mine):
                if result is not None:
                    r = 8 * (n * (result.shape[0] // 8) // len(mine))
                    order["pace"] = result[r:r + 8, 0:128]
                next(sides[k][0], None)
                order["pace"] = None
        for gen, _ in (main, *sides):
            for _ in gen:
                pass

    def tied(ref, tiles, start, size):
        tokens, order["tokens"] = order["tokens"], []
        cols = [ref[j, pl.ds(start // 2, size // 2), :] for j in tiles]
        parts = [cols[-1][r:r + 8] for r in range(0, size // 2, 8)]
        for i, token in enumerate(tokens):
            r = (2 * i + 1) * len(parts) // (2 * len(tokens))
            parts[r] = jnp.where(order["zero"] != 0, pltpu.bitcast(token, U32), parts[r])
        cols[-1] = jnp.concatenate(parts, axis=0)
        return jnp.concatenate([pltpu.bitcast(v, BF) for v in cols], axis=1)

    def to_freq(x):
        y = [v.astype(BF) for v in _radix5(x)]
        f = [_dot(jnp.concatenate(y[j:j + 2], axis=1),
                  jnp.concatenate([_get(dmat, 2 * j - 1 + 2 * b + a) for a in (0, 1)], axis=0))
             for j in (1, 3) for b in (0, 1)]
        return [_dot(y[0], _get(dmat, 0))] + f

    def input_rows(i, r, n):
        return [xio[i, r // 8:(r + n) // 8, :, _tile(j)].astype(F32).reshape(n, 128)
                for j in range(NT)]

    def input_freq(j, r, n):
        return xf0[r // SLAB % 2][j, pl.ds(r // T * SLAB + r % SLAB, n), :]

    def to_natural(g):
        for r in range(0, T, 32):
            rr = pl.ds(g * T + r, 32)
            for j, v in enumerate(_regroup([x[0, rr, :] for x in xres])):
                wtmp[j, r:r + 32, :] = v
            written(wtmp)
            if r % 256 == 224:
                yield
        for j in range(NT):
            ubuf[j][4 * g:4 * g + 4] = _dot(
                wtmp[j, 0:T, :].astype(BF), _get(dmat, NFWD + j)).reshape(T // 128, 128, 128)
        yield
        yield
        for r in range(0, T, 16):
            rr = pl.ds(g * T + r, 16)
            y = _feat_inv([ubuf[j][4 * g + r // 128, pl.ds(r % 128, 16), :] for j in range(NT)],
                          _lanes(16) < 64, jnp.where, _roll64)
            for j in range(NT):
                xres[j][0, rr, :] = y[j]
            written(xres[r // 16 % NT])
            if r % 128 == 112:
                yield

    def head_scale(i):
        for r in range(i * SLAB, (i + 1) * SLAB, LN_ROWS):
            paced(xres[0])
            rstd = _layernorm_scale([xres[j][0, r:r + LN_ROWS, :] for j in range(NT)])
            for n in range(0, LN_ROWS, 16):
                scale[0, r + n:r + n + 16, :] = rstd[n:n + 16]
                written(scale)
            yield

    def head_fft(i, tiles=TILES, first=None):
        gate = scale if first is None else scale0[first[1]]
        for j in tiles:
            paced(gate)
            if first is None:
                rs = [pl.ds(i * SLAB + 8 * s1, 8) for s1 in range(R1)]
                u = _tok_fwd([xres[j][0, r, :] * scale[0, r, :] for r in rs], order["tokens"])
            else:
                u = _tok_fwd([xf0[first[1]][j, _ds(first[0] * SLAB + 8 * s1, 8), :]
                              * gate[0, 8 * s1:8 * s1 + 8, :] for s1 in range(R1)], [])
            for part in ((0, 8, 4, 12), (2, 6, 10, 14), (1, 15), (7, 9), (3, 5, 11, 13)):
                if part[0]:
                    written(ubuf[j])
                for c in part:
                    for n in range(2):
                        ubuf[j][c, _ds(n * R2 + 8 * i, 8), :] = u[2 * c + n]
            if first is None:
                step_done(gate, ubuf[j])
            else:
                written(ubuf[j])
            yield

    def tail_fft(i, src, tiles=TILES):
        for j in tiles:
            paced(vbuf[j])
            y = _tok_inv([vbuf[j][cr // 2, pl.ds((cr % 2) * R2 + 8 * i, 8), :] for cr in range(R1)])
            for part in ((0, 4), (2, 4), (1, 8), (5, 8), (3, 4)):
                if part[0]:
                    written(xres[j])
                for s1 in range(part[0], R1, part[1]):
                    r = pl.ds(i * SLAB + 8 * s1, 8)
                    xres[j][0, r, :] = y[s1] + (
                            xres[j][0, r, :] if src is xres else input_freq(j, i * SLAB + 8 * s1, 8))
            step_done(vbuf[TILES[(TILES.index(j) + 1) % NT]], xres[j])
            yield

    def tail_norm(i):
        for r in range(i * SLAB, (i + 1) * SLAB, LN_ROWS):
            paced(xres[0])
            x = [xres[j][0, r:r + LN_ROWS, :] for j in range(NT)]
            rstd = _layernorm_scale(x)
            order["tokens"] += [rstd[n:n + 8] for n in range(0, LN_ROWS, 8)]
            for n in range(0, LN_ROWS, 16):
                for j in range(NT):
                    v = x[j][n:n + 16] * rstd[n:n + 16]
                    if j == 0:
                        v = jnp.where(_lanes(16) == 0, 1.0, v)
                    _put(xn, j, v, r + n)
                written(xn)
            yield

    def head(*slabs):
        return _chain(*[g for i in slabs for g in (head_scale(i), head_fft(i))])

    def tail(src, *slabs):
        return _chain(*[g for i in slabs for g in (tail_fft(i, src), tail_norm(i))])

    n_tok = SLAB // LN_ROWS + NT

    def make_perm():
        word = _rows(64)
        c = word >> 2
        for part in range(2):
            for u in range(2):
                hot = 0
                for n in range(2):
                    j = 2 * (word & 1) + n
                    plus, minus = c + R1 * j, R1 - c + R1 * (3 - j)
                    if part:
                        plus, minus = jnp.where(c == 0, plus + NCLS, plus), minus & 127
                    else:
                        minus = jnp.where(c == 0, minus - NCLS, minus)
                    src = jnp.where(((word >> 1) & 1) == u, plus, minus)
                    hot = hot | jnp.where(src == _lanes(64), 0x3A00 << (16 * n), 0)
                perm[2 * part + u] = pltpu.bitcast(hot, U32)

    def filter_block(b, slot):
        for a in range(2):
            for u in range(2):
                wpair[a, u, 0:DF // 2, :] = pltpu.bitcast(wbuf[a, slot, 0:DF - 1, _tile(u)], U32)

        def half(a, u, res, high):
            v = wpair[a, u, pl.ds(res // 2, 32, stride=5), :]
            if res == 0:
                top = jnp.broadcast_to(wbuf[1 - a, slot, DF - 1:DF, _tile(u)].astype(F32), v.shape)
                v = jnp.where(_rows(32) == 0, pltpu.bitcast(top, U32) >> 16, v)
            if res % 2:
                return (v & np.uint32(0xFFFF0000)) if high else (v >> 16)
            return (v << 16) if high else (v & np.uint32(0xFFFF))

        stacks = [[(a, j), (a, j + 1)] for j in (1, 3) for a in range(2)] + [[(0, 0), (1, 0)]]
        for n, parts in enumerate(stacks):
            o = [_dot_nt(tied(perm, [2 * (b // 4) + u], 0, 128), jnp.concatenate(
                [pltpu.bitcast(half(a, u, RESIDUES[j][0], False)
                               | half(a, u, RESIDUES[j][1], True), BF) for a, j in parts],
                axis=0)) for u in range(2)]
            low = (_rows(128) & 4) == 0
            coef[n, :, _ds(8 * b, 8), :] = jnp.where(low, o[0], o[1]).reshape(NCLS, 8, 128)
            coef[NT + n, :, _ds(8 * (7 - b), 8), :] = jnp.where(low, o[1], o[0]).reshape(
                NCLS, 8, 128)
            yield o[0]

    def filter_finish():
        for n in range(NT, 2 * NT):
            v = coef[n, 0, 0:32, :]
            coef[n, 0, 0:32, :] = jnp.where((_rows(32) & 3) == 0, pltpu.roll(v, 4, 0), v)
        for c in range(NCLS):
            _put(smat, NCLS + c, _get(smat, c).T)

    def filter_tile0(c, z, again):
        if not again:
            lane = _lanes(R2)
            first = lane <= 64
            sign = jnp.where((lane & 63) == 0, 0.0, jnp.where(first, -1.0, 1.0))
            plus, minus = coef[NT - 1, c], coef[2 * NT - 1, c]
            sets = [(c, plus + minus), (NCLS + c, plus - minus)]
            if c == 0:
                sets = [(n, jnp.where(_rows(R2) == 0, a, b)) for n, a, b in (
                    (0, plus, sets[0][1]), (NCLS, 0.0, sets[1][1]), (2 * NCLS, minus, sets[0][1]))]
            for n, v in sets:
                a, b = (_roll64(v), v) if n // NCLS == 1 else (v, _roll64(v))
                coef0[0, n] = jnp.where(lane == 0, 0.0, jnp.where(first, a, b))
                coef0[1, n] = sign * jnp.where(first, b, a)
        p, q = z[0:R2], z[R2:]
        rp, rq = _roll64(p), _roll64(q)
        a1, a2, b1, b2, c1, c2 = (coef0[t, n] for n in (c, NCLS + c, c or 2 * NCLS) for t in (0, 1))
        return jnp.concatenate([(p * a1 + rp * a2) + (rq * b2 - q * b1),
                                (q * c1 + rq * c2) + (p * b1 - rp * b2)], axis=0)

    def filter_pair(c, z, pair):
        pr, pi, qr, qi = (z[h, _tile(t)] for h in (slice(0, R2), slice(R2, None)) for t in (0, 1))
        ur, ui, vr, vi = (coef[n + 2 * pair, c] for n in (0, 1, NT, NT + 1))
        xr, xi, yr, yi = pr - qi, pi + qr, pr + qi, pi - qr
        xr, xi = xr * ur - xi * ui, xr * ui + xi * ur
        yr, yi = yr * vr - yi * vi, yr * vi + yi * vr
        out = [xr + yr, xi + yi, xi - yi, yr - xr]
        if c == 0:
            real = [pr * ur - pi * ui, pr * ui + pi * ur, qr * vr - qi * vi, qr * vi + qi * vr]
            out = [jnp.where(_rows(R2) == 0, a, b) for a, b in zip(real, out)]
        return jnp.concatenate([jnp.concatenate(out[h:h + 2], axis=1) for h in (0, 2)], axis=0)

    def spectral_mid(again):
        items = []
        for n in range(2 * NCLS):
            items.append(((1, 2) if n < NCLS else (3, 4), n % NCLS))
            items += [((0,), n - NCLS // 2)] * (0 <= n - NCLS // 2 < NCLS)
        z, y = {}, {}
        for n in range(len(items) + 2 * LAG):
            if n < len(items):
                tiles, c = items[n]
                z[n] = _dot(tied(smat, [c], 0, 128),
                            jnp.concatenate([ubuf[j][c] for j in tiles], axis=1).astype(BF))
            if 0 <= n - LAG < len(items):
                tiles, c = items[n - LAG]
                y[n - LAG] = (filter_pair(c, z[n - LAG], tiles[0] // 2) if tiles[0]
                              else filter_tile0(c, z[n - LAG], again)).astype(BF)
            if n >= 2 * LAG:
                tiles, c = items[n - 2 * LAG]
                v = _dot(_get(smat, NCLS + c), y[n - 2 * LAG])
                for t, j in enumerate(tiles):
                    vbuf[j][c] = v[:, _tile(t)]
            yield z.get(n)

    def head_minor(j):
        return jnp.concatenate([rows[j, pl.ds(d, H, stride=DH), :] for d in range(DH)], axis=0)

    def project_weight(i):
        for e in range(NT):
            paced(wraw[i])
            for r in range(0, 64, 16):
                y = _feat_fwd_halves([wraw[i][e, 64 * t + r:64 * t + r + 16, :].astype(F32)
                                      for t in range(10)])
                if r:
                    written(wtmp)
                for t in range(10):
                    wtmp[e, 64 * t + r:64 * t + r + 16, :] = y[t]
            step_done(wraw[i], wtmp)
            yield
        f = [_dot(_get(dmat, NFWD + j), jnp.concatenate(
            [wtmp[e, _tile(j), :] for e in range(NT)], axis=1).astype(BF)) for j in range(NT)]
        dc = lax.broadcasted_iota(jnp.int32, (8, D), 0) == 0
        f[0] = jnp.concatenate([jnp.where(dc, 0.0, f[0][0:8]), f[0][8:]], axis=0)
        f = [f[0]] + [jnp.concatenate([f[j][h:h + 64], f[j + 1][h:h + 64]], axis=0)
                      for j in (1, 3) for h in (0, 64)]
        for j in range(NT):
            if i == 0:
                rows[j, 0:D, :] = f[j].astype(BF).T.astype(F32)
                _put(wqt, j, head_minor(j))
            elif i == 1:
                _put(wkt, j, f[j].astype(BF).T)
            else:
                for e in range(NT):
                    _put(wvf, e, f[j][:, _tile(e)], 128 * j)
            written((wqt, wkt, wvf)[i])
            yield

    def project_wo():
        for r in range(0, D, 128):
            f = to_freq([wraw[3][j, r:r + 128, :].astype(F32) for j in range(NT)])
            for j in range(NT):
                _put(wof, j, f[j], r)
            written(wof)
            yield

    def keys(*blocks):
        for u in blocks:
            k = _dot_nt(tied(wkt, range(NT), 0, D), _cat(xn, (128 * u, 128)))
            p = _phi(k)
            _put(pk, u % 8, p)
            yield k

    def key_sums(g):
        for j in range(NT):
            v = _dot(tied(pk, [u % 8 for u in range(4 * g, 4 * g + 4)], 0, D),
                     _get(xn, j, rows=(g * T, T)))
            gacc[j] = gacc[j] + v if g else v
            yield v

    def mix(last):
        rows[NT, 0:D, :] = gacc[0]
        z = head_minor(NT)
        zh = z.astype(BF)
        zl = (z - zh.astype(F32)).astype(BF)
        zrow[...] = _dot_nt(jnp.tile(jnp.where(_lanes(16) == 0, 1.0, 0.0), (1, 2)).astype(BF), jnp.concatenate([zh, zl], axis=1))
        kvs, done = [], 0
        for e in range(NT):
            a = (128 * e) // DH * DH // 16 * 16
            b = -(-(((128 * e + 127) // DH + 1) * DH) // 16) * 16
            kv = _dot(jnp.concatenate([gacc[j, a:b, :] for j in range(NT)], axis=1).astype(BF),
                         _get(wvf, e))
            head = lambda ax, off: ((lax.broadcasted_iota(jnp.int32, kv.shape, ax) + off)
                                    * 3277) >> 16
            kvs.append((a, b, jnp.where(head(0, a) == head(1, 128 * e), kv, 0.0).astype(BF)))
        yield
        for e, (a, b, kv) in enumerate(kvs):
            m = _dot(kv, jnp.concatenate([wraw[3][j, _tile(e), :] for j in range(NT)], axis=1)
                     if last else _cat(wof, (128 * e, 128)))
            for j in range(NT):
                if done > a:
                    rows[j, a:done, :] += m[0:done - a, _tile(j)]
                rows[j, done:b, :] = m[done - a:, _tile(j)]
            done = b
        yield
        for j in range(NT):
            _put(mmat, j, head_minor(j))
        yield

    def project_q(*slabs):
        r, n = slabs[0] * SLAB, len(slabs) * SLAB
        for j in range(NT):
            q = _dot_nt(tied(xn, range(NT), r, n), _cat(wqt, (128 * j, 128)))
            pq[j, r:r + n, :] = _phi(q)
            yield q

    def normalize(*slabs):
        for r in range(slabs[0] * SLAB, (slabs[-1] + 1) * SLAB, 64):
            p = [pq[j, r:r + 64, :] for j in range(NT)]
            den = [p[j] * zrow[0:1, _tile(j)] for j in range(NT)]
            den = sum(den[1:], den[0])
            den = den + pltpu.roll(den, 64, 1)
            den = den + pltpu.roll(den, 32, 1)
            inv = 1.0 / (den + 1e-6)
            order["tokens"] += [inv[n:n + 8] for n in range(0, 64, 8)]
            for i in range(0, 64, 16):
                for j in range(NT):
                    _put(att, j, p[j][i:i + 16] * inv[i:i + 16], r + i)
                written(att)
            yield

    def attend(last, *slabs):
        r, n = slabs[0] * SLAB, len(slabs) * SLAB
        for j in range(NT):
            v = _dot(tied(att, range(NT), r, n), _get(mmat, j))
            x = xres[j][0, r:r + n, :] + v
            if last:
                for m, i in enumerate(slabs):
                    xio[i, :, :, _tile(j)] = x[m * SLAB:(m + 1) * SLAB].reshape(
                        R1, 8, 128).astype(BF)
                for i in slabs:
                    if (i, j) in o_copy:
                        o_copy[i, j].start()
            else:
                xres[j][0, r:r + n, :] = x
            yield v

    def first_slabs(k, carry):
        @pl.when(k + 1 < NG)
        def _():
            for c in slab_copies(2 * k + 2) + slab_copies(2 * k + 3):
                c.start()

        @pl.when(k + 1 == NG)
        def _():
            w_copy[1].start()

        for odd in range(2):
            i = 2 * k + odd
            slab_copies(i, (0,))[0].wait()

            @pl.when(i > 0)
            def _():
                for c in slab_copies(i - 1, (1, 2)):
                    c.wait()

            f = to_freq(input_rows(i, 0, SLAB))
            for j in range(NT):
                xf0[odd][j, _ds(k * SLAB, SLAB), :] = f[j]
            scale0[odd][0] = _layernorm_scale(f)
            prev = (k if odd else (k + NG - 1) % NG, 1 - odd)
            emit((head_fft((i + NS - 1) % NS, first=prev), 1))
            order["tokens"] = []
            emit((filter_block((i + NS - 1) % NS, i), 1))
            order["results"] = []
        return carry

    for c in [w_copy[0], *slab_copies(0, (0,))]:
        c.start()
    make_perm()
    xf0[1][:, (NG - 1) * SLAB:, :] = jnp.zeros((NT, SLAB, 128), F32)
    wbuf[:, 0] = jnp.zeros((2, DF, 256), BF)
    scale0[1][0] = jnp.zeros((SLAB, 128), F32)
    w_copy[0].wait()
    for c in slab_copies(0, (1, 2)) + slab_copies(1):
        c.start()
    probe = pltpu.bitcast(dmat[0, 0:8, :], jnp.int32)[0, 0]
    order["zero"] = probe ^ int(_DMAT.view(np.int32)[0, 0, 0])
    lax.fori_loop(0, NG, first_slabs, 0)
    for c in w_copy[2:]:
        c.start()
    for c in slab_copies(NS - 1, (1, 2)):
        c.wait()
    emit((filter_block(NS - 1, NS), 1))
    emit((head_fft(NS - 1, (1, 2), (NG - 1, 1)), 1))
    w_copy[1].wait()
    filter_finish()
    late = head_fft(NS - 1, (0, 3, 4), (NG - 1, 1))
    for layer in range(2):
        src, last = (xres if layer else xf0), layer == 1
        extra = [iter(()) if last else project_weight(i) for i in (1, 0, 2)]
        order["tokens"] = []
        mid = spectral_mid(last)
        emit((_take(mid, 8), 8), (_take(late, 2), 2))
        emit((_take(mid, 12), 12), (late, 3))
        for c in w_copy[2:3 + NT] * (not last):
            c.wait()
        emit((_take(mid, 4 + 2 * LAG), 4 + 2 * LAG), (_take(extra[0], 3), 3))
        emit((_take(mid, 16), 16), (extra[0], 2 * NT - 3),
             (_chain(tail_fft(0, src, (1, 2)), tail_fft(1, src, (1, 2))), 4))
        emit((mid, 8 - LAG), (_chain(tail_fft(0, src, (0,)), tail_fft(1, src, (0,))), 2))
        lead = _chain(tail_fft(0, src, (3, 4)), tail_norm(0))
        if last:
            pl.semaphore_signal(sem_f, 1)
            pl.semaphore_wait(sem_f, 1)
        else:
            for c in w_copy[3 + NT:]:
                c.wait()
            emit((project_wo(), 1))
        emit((lead, 1))
        order["tokens"] = []
        side, n = _chain(tail_fft(1, src, (3, 4)), tail_norm(1)), 1
        emit((keys(0), 1), (_take(side, n), n))
        emit((keys(1), 1), (side, 4 - n))
        main = _chain(keys(2, 3), *[s for g in range(NG - 1) for s in (
            key_sums(g), keys(*range(4 * g + 4, 4 * g + 8)))])
        emit((_take(main, 7), 7 + last), (tail(src, 2, 3), 2 * n_tok))

        def middle():
            emit((_take(main, 9), 10), (tail(src, 4, 5), 2 * n_tok))
            emit((_take(main, 9), 9 + last), (tail(src, 6, 7), 2 * n_tok))

        if last:
            middle()
        else:
            pl.when(order["zero"] == 0)(middle)
            order["tokens"], order["results"] = [], []
        first = project_q(0, 1)
        if last:
            side, n = _chain(*map(to_natural, range(NG))), 19
        else:
            side, n = _chain(*extra[1:]), 4 * NT
        emit((_chain(main, _take(first, last), key_sums(NG - 1)), 9 + last),
             (_take(side, n), n))
        plan = [((first, NT - last), (mix(last), 3)),
                ((project_q(2, 3), NT), (normalize(0, 1), 8)),
                ((attend(last, 0, 1), NT), (normalize(2, 3), 8)),
                ((project_q(4, 5), NT),),
                ((attend(last, 2, 3), NT), (normalize(4, 5), 8))]
        if last:
            share = (5, 0, 2, 2, 0, 4, 0, 0, 0)
            plan += [((project_q(6, 7), NT),),
                     ((attend(last, 4, 5), NT), (normalize(6, 7), 8)),
                     ((attend(last, 6), NT),)]
        else:
            side = _chain(head(*range(NS - 2)), head_scale(NS - 2), head_fft(NS - 2, (1, 2, 0)))
            share = (0, 0, 0, 12, 2, 14, 7, 4, 3, 5)
            plan += [((attend(last, 4, 5), NT),),
                     ((project_q(6), NT),),
                     ((project_q(7), NT), (normalize(6), 4)),
                     ((attend(last, 6), NT), (normalize(7), 4))]
        plan.append(((attend(last, 7), NT),))
        for streams, n in zip(plan, share):
            emit(*streams, (_take(side, n), n))
        if not last:
            emit((_chain(side, head_scale(NS - 1), head_fft(NS - 1, (1, 2))), 1))
            late = _chain(head_fft(NS - 1, (0, 3, 4)), head_fft(NS - 2, (3, 4)))
    for c in o_copy.values():
        c.wait()


@jax.jit
def pallas_interleave_layers__spectral_gfnet__linear_attn_block__prompt_kernel(
    A_x: jax.Array,
    A_w_r: jax.Array,
    A_w_i: jax.Array,
    B_x: jax.Array,
    B_wqkv: jax.Array,
    B_wo: jax.Array,
):
    del B_x
    vmem = pltpu.VMEM
    out = pl.pallas_call(
        _kernel,
        out_shape=jax.ShapeDtypeStruct((R1, R2, D), BF),
        in_specs=[pl.BlockSpec(memory_space=pl.ANY)] * 7,
        out_specs=pl.BlockSpec(memory_space=pl.ANY),
        scratch_shapes=[
            vmem((NS, R1, 8, D), BF),
            vmem((2, NS + 1, DF, 256), BF),
            [vmem((NT + 1, D, 128), BF)] * 4,
            vmem((2 * NCLS, 64, 128), U32), vmem(_DMAT.shape, U32), vmem((4, 64, 128), U32),
            vmem((2, 2, DF // 2 + 8, 128), U32),
            vmem((2 * NT, NCLS, R2, 128), F32),
            vmem((2, 2 * NCLS + 1, R2, 128), F32),
            [vmem((NT, S // 2, 128), F32)] * 2,
            [vmem((2, S, 128), F32)] * NT,
            vmem((NT, S // 2, 128), U32), vmem((2, S, 128), F32),
            [vmem((NCLS, 128, 128), F32)] * NT,
            [vmem((NCLS + 1, 128, 128), F32)] * NT,
            *[vmem((NT, D // 2, 128), U32)] * 4,
            vmem((NT, D, 128), F32),
            vmem((NT + 1, D + 24, 128), F32),
            vmem((NT, D // 2, 128), U32), vmem((16, D), F32),
            vmem((8, D // 2, 128), U32), vmem((NT, S // 2, 128), U32),
            vmem((NT, D, 128), F32),
            vmem((NT, S, 128), F32),
            [vmem((2, SLAB, 128), F32)] * 2,
            pltpu.SemaphoreType.DMA((3 * NS,)),
            pltpu.SemaphoreType.DMA((3 + 4 * NT,)),
            pltpu.SemaphoreType.DMA((NS + NT - 1,)),
            pltpu.SemaphoreType.REGULAR,
        ],
        compiler_params=pltpu.CompilerParams(vmem_limit_bytes=100 * 1024 * 1024),
    )(A_x.reshape(R1, R2, D), A_w_r.T, A_w_i.T, B_wqkv, B_wo, _SMAT, _DMAT)
    return out.reshape(1, S, D)
```
